```python
import jax
import jax.numpy as jnp

def _softmax(x, axis=-1):
    return jax.nn.softmax(x, axis=axis)
def _gelu(x):
    return jax.nn.gelu(x, approximate=True)
def _silu(x):
    return jax.nn.silu(x)
def _sigmoid(x):
    return jax.nn.sigmoid(x)
def _layernorm(x, axis=-1, eps=1e-5):
    m = jnp.mean(x, axis=axis, keepdims=True)
    v = jnp.var(x, axis=axis, keepdims=True)
    return (x - m) / jnp.sqrt(v + eps)
def _scatter_add(tgt, idx, src, axis=0):
    return tgt.at[idx].add(src)
def _segment_sum(src, seg, n):
    return jax.ops.segment_sum(src, seg, n)
class _Rng:
    def __init__(self, key):
        self._k = key
    def _next(self):
        self._k, sub = jax.random.split(self._k)
        return sub
    def normal(self, shape):
        return jax.random.normal(self._next(), shape, dtype=jnp.bfloat16)
    def randint(self, lo, hi, shape):
        return jax.random.randint(self._next(), shape, lo, hi, dtype=jnp.int32)
    def uniform(self, shape, lo=0.0, hi=1.0):
        return jax.random.uniform(self._next(), shape, jnp.bfloat16, lo, hi)
    def permutation(self, n):
        return jax.random.permutation(self._next(), n)


kernel_name = 'gated_mix__mha_block_cached__compressed_kv_cla__decode'

def setup_inputs():
    _rng = _Rng(jax.random.key(int.from_bytes(__import__("os").urandom(4), "little")))
    _w = (lambda a: (lambda t: t.astype(jnp.bfloat16) if jnp.issubdtype(t.dtype, jnp.floating) else t)(jnp.asarray(a)))
    def _A_setup():
        B, Sq, D = 2, 1, 512
        H, Sk, Dh = 32, 8192, 128
        return {
            "x": _w((lambda *s: _rng.normal(s) * 0.05)(B, Sq, D)),
            "k_cache": _w((lambda *s: _rng.normal(s) * 0.05)(B, H, Sk, Dh)),
            "v_cache": _w((lambda *s: _rng.normal(s) * 0.05)(B, H, Sk, Dh)),
            "wq": _w((lambda *s: _rng.normal(s) * 0.05)(D, H * Dh) * (D ** -0.5)),
            "wo": _w((lambda *s: _rng.normal(s) * 0.05)(H * Dh, D) * ((H * Dh) ** -0.5)),
        }
    _A_in = _A_setup()

    def _B_setup():
        B, H, Sq, Sk, D, M = 2, 32, 1, 8192, 128, 512
        Dc = 4 * D
        return {
            "x": _w((lambda *s: _rng.normal(s) * 0.05)(B, Sq, M)),
            "c_kv": _w((lambda *s: _rng.normal(s) * 0.05)(B, Sk, Dc)),
            "w_q": _w((lambda *s: _rng.normal(s) * 0.05)(M, H, D) * (M ** -0.5)),
            "w_uk": _w((lambda *s: _rng.normal(s) * 0.05)(Dc, H, D) * (Dc ** -0.5)),
            "w_uv": _w((lambda *s: _rng.normal(s) * 0.05)(Dc, H, D) * (Dc ** -0.5)),
            "w_o": _w((lambda *s: _rng.normal(s) * 0.05)(H, D, M) * ((H * D) ** -0.5)),
        }
    _B_in = _B_setup()

    return {
        "A_x": _A_in["x"],
        "A_k_cache": _A_in["k_cache"],
        "A_v_cache": _A_in["v_cache"],
        "A_wq": _A_in["wq"],
        "A_wo": _A_in["wo"],
        "B_x": _B_in["x"],
        "B_c_kv": _B_in["c_kv"],
        "B_w_q": _B_in["w_q"],
        "B_w_uk": _B_in["w_uk"],
        "B_w_uv": _B_in["w_uv"],
        "B_w_o": _B_in["w_o"],
        "gate_w": _w((lambda *s: _rng.normal(s) * 0.05)(512)),
    }

def reference(A_x, A_k_cache, A_v_cache, A_wq, A_wo, B_x, B_c_kv, B_w_q, B_w_uk, B_w_uv, B_w_o, gate_w):
    def _A_ref(x, k_cache, v_cache, wq, wo):
        B, Sq, D = x.shape
        H, Dh = 32, 128
        q = (lambda x, *d: x.transpose(*d))((x @ wq).reshape(B, Sq, H, Dh), 0, 2, 1, 3)
        scores = jnp.einsum("bhqd,bhkd->bhqk", q, k_cache) * (Dh ** -0.5)
        p = _softmax(scores, axis=-1)
        o = jnp.einsum("bhqk,bhkd->bhqd", p, v_cache)
        return (lambda x, *d: x.transpose(*d))(o, 0, 2, 1, 3).reshape(B, Sq, H * Dh) @ wo

    def _B_ref(x, c_kv, w_q, w_uk, w_uv, w_o):
        B, Sq, M = x.shape[0], x.shape[1], x.shape[2]
        Sk = c_kv.shape[1]
        H, D = w_q.shape[1], w_q.shape[2]
        q = jnp.einsum("bqm,mhd->bhqd", x, w_q)
        k = jnp.einsum("bkc,chd->bhkd", c_kv, w_uk)
        v = jnp.einsum("bkc,chd->bhkd", c_kv, w_uv)
        scores = jnp.einsum("bhqd,bhkd->bhqk", q, k) * (D ** -0.5)
        off = Sk - Sq
        qi = jnp.arange(Sq)[:, None]
        kj = jnp.arange(Sk)[None, :]
        cmask = kj <= (qi + off)
        scores = jnp.where(cmask[None, None], scores, -1e9)
        p = _softmax(scores, axis=-1)
        ctx = jnp.einsum("bhqk,bhkd->bhqd", p, v)
        return jnp.einsum("bhqd,hdm->bqm", ctx, w_o)

    x = A_x
    g = _sigmoid((x * gate_w).sum(-1, keepdims=True))
    a = _A_ref(x, A_k_cache, A_v_cache, A_wq, A_wo)
    b = _B_ref(x, B_c_kv, B_w_q, B_w_uk, B_w_uv, B_w_o)
    return g * a + (1 - g) * b
```

```python
import jax
import jax.numpy as jnp
import jax.experimental.pallas as pl
import jax.experimental.pallas.tpu as pltpu

_B, _H, _SK, _DH, _DM, _DC = 2, 32, 8192, 128, 512, 512
_NBH = _B * _H
_LOG2E = 1.4426950408889634
_SCALE = _DH ** -0.5

_NBUF = 4
_KV_PIECE = 192
_CKV_CHUNK = 1024


def _pieces(total, piece):
    out, off = [], 0
    while off < total:
        n = min(piece, total - off)
        out.append((off, n))
        off += n
    return out


def _nt_dot(a, b):
    return jax.lax.dot_general(a, b, (((1,), (1,)), ((), ())),
                               preferred_element_type=jnp.float32)


def _dot(a, b):
    return jnp.dot(a, b, preferred_element_type=jnp.float32)


def _kernel(x_hbm, kc_hbm, vc_hbm, awq_hbm, awo_hbm, ckv_hbm, bwq_hbm, wuk_hbm,
            wuv_hbm, bwo_hbm, gw_hbm, o_ref,
            x_v, gw_v, awq_v, awo_v, ckv_v, bwq_v, wuk_v, wuv_v, bwo_v,
            kbuf, vbuf, stack_v, q3_v, acco_v, wsem, ksem, vsem):
    bf16, f32 = jnp.bfloat16, jnp.float32

    def start_rows(src, dst, sem, rows, piece, base=0):
        n_full = rows // (2 * piece)

        def body(i, c):
            for p in range(2):
                off = pl.multiple_of((2 * i + p) * piece, 16)
                pltpu.make_async_copy(src.at[pl.ds(base + off, piece)],
                                      dst.at[pl.ds(off, piece)], sem).start(priority=p)
            return c
        jax.lax.fori_loop(0, n_full, body, 0)
        rest = rows - n_full * 2 * piece
        for j, (off, n) in enumerate(_pieces(rest, piece)):
            o = n_full * 2 * piece + off
            pltpu.make_async_copy(src.at[pl.ds(base + o, n)], dst.at[pl.ds(o, n)],
                                  sem).start(priority=j % 2)

    def wait_all(dst, sem):
        pltpu.make_async_copy(dst, dst, sem).wait()

    def issue_head(i, slot):
        base = i * _SK
        for off, n in _pieces(_SK, _KV_PIECE):
            pltpu.make_async_copy(kc_hbm.at[pl.ds(base + off, n)],
                                  kbuf.at[slot, pl.ds(off, n)], ksem.at[slot]).start(priority=0)
            pltpu.make_async_copy(vc_hbm.at[pl.ds(base + off, n)],
                                  vbuf.at[slot, pl.ds(off, n)], vsem.at[slot]).start(priority=1)

    pltpu.make_async_copy(x_hbm, x_v, wsem.at[0]).start()
    pltpu.make_async_copy(gw_hbm, gw_v, wsem.at[1]).start()
    start_rows(bwq_hbm, bwq_v, wsem.at[2], 16384, 192)
    start_rows(wuk_hbm, wuk_v, wsem.at[3], 16384, 192)
    start_rows(ckv_hbm, ckv_v.at[0], wsem.at[4], _SK, 48, base=0)
    start_rows(ckv_hbm, ckv_v.at[1], wsem.at[5], _SK, 48, base=_SK)
    start_rows(wuv_hbm, wuv_v, wsem.at[6], 16384, 192)
    start_rows(bwo_hbm, bwo_v, wsem.at[7], 4096, 48)
    start_rows(awq_hbm, awq_v, wsem.at[8], 512, 16)
    start_rows(awo_hbm, awo_v, wsem.at[9], 4096, 48)
    for s in range(_NBUF):
        issue_head(s, s)

    row256 = jax.lax.broadcasted_iota(jnp.int32, (256, 128), 0)
    lane256 = jax.lax.broadcasted_iota(jnp.int32, (256, 128), 1)
    diag256 = (row256 & 31) == (lane256 & 31)
    row128 = jax.lax.broadcasted_iota(jnp.int32, (128, 128), 0)
    lane128 = jax.lax.broadcasted_iota(jnp.int32, (128, 128), 1)

    def expand(cst, w2_ref):
        def body(s, acc):
            e_s = (row128 == 4 * s + (lane128 >> 5)).astype(bf16)
            y = jnp.where(diag256, _dot(cst, e_s), 0.0).astype(bf16)
            for j in range(4):
                r0 = pl.multiple_of((32 * j + s) * 128, 128)
                acc = acc + _dot(y[64 * j:64 * j + 64], w2_ref[pl.ds(r0, 128), :])
            return acc
        return jax.lax.fori_loop(0, 32, body, jnp.zeros((64, 128), f32))

    def absorb(q, w2_ref):
        def body(s, acc):
            ts = []
            for j in range(4):
                r0 = pl.multiple_of((32 * j + s) * 128, 128)
                ts.append(_nt_dot(q, w2_ref[pl.ds(r0, 128), :]))
            t = jnp.where(diag256, jnp.concatenate(ts, axis=0), 0.0).astype(bf16)
            g_s = (lane128 == 4 * s + (row128 >> 5)).astype(bf16)
            return acc + _dot(t, g_s)
        return jax.lax.fori_loop(0, 32, body, jnp.zeros((256, 128), f32))

    wait_all(x_v, wsem.at[0])
    row8 = jax.lax.broadcasted_iota(jnp.int32, (8, _DM), 0)
    x0 = x_v[0].astype(f32)
    x1 = x_v[1].astype(f32)
    x8 = jnp.where(row8 == 0, jnp.broadcast_to(x0, (8, _DM)),
                   jnp.where(row8 == 1, jnp.broadcast_to(x1, (8, _DM)), 0.0))
    row64 = jax.lax.broadcasted_iota(jnp.int32, (64, 128), 0)
    for j in range(4):
        xa = jnp.broadcast_to(x0[:, 128 * j:128 * j + 128], (64, 128))
        xb = jnp.broadcast_to(x1[:, 128 * j:128 * j + 128], (64, 128))
        stack_v[64 * j:64 * j + 64, :] = jnp.where(row64 < 32, xa, xb).astype(bf16)
    wait_all(bwq_v, wsem.at[2])
    q_b = expand(stack_v[...], bwq_v).astype(bf16)
    wait_all(wuk_v, wsem.at[3])
    stack_v[...] = absorb(q_b, wuk_v).astype(bf16)

    qa = [jnp.concatenate([stack_v[64 * j + 32 * b:64 * j + 32 * b + 32, :] for j in range(4)], axis=1)
          for b in range(_B)]
    for b in range(_B):
        wait_all(ckv_v.at[b], wsem.at[4 + b])

        def bstep(t, carry, b=b):
            m, l, acc = carry
            c = ckv_v[b, pl.ds(pl.multiple_of(t * _CKV_CHUNK, _CKV_CHUNK), _CKV_CHUNK), :]
            s = _nt_dot(qa[b], c) * _SCALE
            m_new = jnp.maximum(m, jnp.max(s, axis=1, keepdims=True))
            alpha = jnp.exp(m - m_new)
            p = jnp.exp(s - m_new)
            l = alpha * l + jnp.sum(p, axis=1, keepdims=True)
            acc = alpha * acc + _dot(p.astype(bf16), c)
            return m_new, l, acc
        init = (jnp.full((32, 1), -1e30, f32), jnp.zeros((32, 1), f32), jnp.zeros((32, _DC), f32))
        _, l, acc = jax.lax.fori_loop(0, _SK // _CKV_CHUNK, bstep, init)
        ctx_c = (acc / l).astype(bf16)
        for j in range(4):
            stack_v[64 * j + 32 * b:64 * j + 32 * b + 32, :] = ctx_c[:, 128 * j:128 * j + 128]

    wait_all(wuv_v, wsem.at[6])
    ctx = expand(stack_v[...], wuv_v)
    wait_all(bwo_v, wsem.at[7])
    row8s = jax.lax.broadcasted_iota(jnp.int32, (8, 128), 0)
    out_b = jnp.zeros((8, _DM), f32)
    for h in range(_H):
        lhs = jnp.where(row8s == 0, jnp.broadcast_to(ctx[h:h + 1], (8, 128)),
                        jnp.where(row8s == 1, jnp.broadcast_to(ctx[32 + h:33 + h], (8, 128)), 0.0))
        out_b = out_b + _dot(lhs.astype(bf16), bwo_v[128 * h:128 * h + 128, :])

    wait_all(awq_v, wsem.at[8])
    q_a = _dot(x8.astype(bf16), awq_v[...]).astype(bf16).astype(f32)
    for b in range(_B):
        for h in range(_H):
            q3_v[b * _H + h] = jnp.broadcast_to(q_a[b:b + 1, 128 * h:128 * h + 128], (8, 128))
    acco_v[...] = jnp.zeros(acco_v.shape, f32)
    wait_all(awo_v, wsem.at[9])

    def head_step(i, carry):
        slot = i % _NBUF
        b = i // _H
        h = i % _H
        q = q3_v[i].astype(bf16)
        pltpu.make_async_copy(kbuf.at[slot], kbuf.at[slot], ksem.at[slot]).wait()
        s = _nt_dot(q, kbuf[slot])
        m = jnp.max(s, axis=1, keepdims=True)
        p = jnp.exp2((s - m) * (_SCALE * _LOG2E))
        l = jnp.sum(p, axis=1, keepdims=True)
        pltpu.make_async_copy(vbuf.at[slot], vbuf.at[slot], vsem.at[slot]).wait()
        o = _dot(p.astype(bf16), vbuf[slot]) / l

        @pl.when(i + _NBUF < _NBH)
        def _():
            issue_head(i + _NBUF, slot)

        wo = awo_v[pl.ds(pl.multiple_of(h * 128, 128), 128), :]
        acco_v[b] = acco_v[b] + _dot(o.astype(bf16), wo)
        return carry
    jax.lax.fori_loop(0, _NBH, head_step, 0)

    wait_all(gw_v, wsem.at[1])
    gw = gw_v[...].astype(f32).reshape(1, _DM)
    g = jax.nn.sigmoid(jnp.sum(x8 * gw, axis=1, keepdims=True))
    for b in range(_B):
        gb = g[b:b + 1]
        res = gb * acco_v[b, 0:1, :] + (1.0 - gb) * out_b[b:b + 1]
        o_ref[b] = res.astype(o_ref.dtype)


@jax.jit
def pallas_gated_mix__mha_block_cached__compressed_kv_cla__decode_kernel(
    A_x: jax.Array,
    A_k_cache: jax.Array,
    A_v_cache: jax.Array,
    A_wq: jax.Array,
    A_wo: jax.Array,
    B_x: jax.Array,
    B_c_kv: jax.Array,
    B_w_q: jax.Array,
    B_w_uk: jax.Array,
    B_w_uv: jax.Array,
    B_w_o: jax.Array,
    gate_w: jax.Array,
):
    del B_x
    bf16, f32 = jnp.bfloat16, jnp.float32
    kc = A_k_cache.reshape(_NBH * _SK, _DH)
    vc = A_v_cache.reshape(_NBH * _SK, _DH)
    ckv = B_c_kv.reshape(_B * _SK, _DC)
    bwq = B_w_q.reshape(_DM * _H, _DH)
    wuk = B_w_uk.reshape(_DC * _H, _DH)
    wuv = B_w_uv.reshape(_DC * _H, _DH)
    bwo = B_w_o.reshape(_H * _DH, _DM)

    any_spec = pl.BlockSpec(memory_space=pl.ANY)
    scratch = [
        pltpu.VMEM((_B, 1, _DM), bf16),
        pltpu.VMEM((_DM,), bf16),
        pltpu.VMEM((_DM, _H * _DH), bf16),
        pltpu.VMEM((_H * _DH, _DM), bf16),
        pltpu.VMEM((_B, _SK, _DC), bf16),
        pltpu.VMEM((_DM * _H, _DH), bf16),
        pltpu.VMEM((_DC * _H, _DH), bf16),
        pltpu.VMEM((_DC * _H, _DH), bf16),
        pltpu.VMEM((_H * _DH, _DM), bf16),
        pltpu.VMEM((_NBUF, _SK, _DH), bf16),
        pltpu.VMEM((_NBUF, _SK, _DH), bf16),
        pltpu.VMEM((256, 128), bf16),
        pltpu.VMEM((_NBH, 8, _DH), f32),
        pltpu.VMEM((_B, 8, _DM), f32),
        pltpu.SemaphoreType.DMA((10,)),
        pltpu.SemaphoreType.DMA((_NBUF,)),
        pltpu.SemaphoreType.DMA((_NBUF,)),
    ]
    return pl.pallas_call(
        _kernel,
        out_shape=jax.ShapeDtypeStruct((_B, 1, _DM), bf16),
        in_specs=[any_spec] * 11,
        out_specs=pl.BlockSpec(memory_space=pltpu.VMEM),
        scratch_shapes=scratch,
        compiler_params=pltpu.CompilerParams(vmem_limit_bytes=100 * 1024 * 1024),
    )(A_x, kc, vc, A_wq, A_wo, ckv, bwq, wuk, wuv, bwo, gate_w)
```

```python
import jax
import jax.numpy as jnp
import jax.experimental.pallas as pl
import jax.experimental.pallas.tpu as pltpu

_B, _H, _SK, _DH, _DM, _DC = 2, 32, 8192, 128, 512, 512
_NBH = _B * _H
_LOG2E = 1.4426950408889634
_SCALE = _DH ** -0.5

_NBUF = 4
_AHEAD = 3
_P256 = 192
_P1K = 48
_CKV_CHUNK = 1024
_NPART = 4
SCOPES = False


def _pieces(total, piece):
    out, off = [], 0
    while off < total:
        n = min(piece, total - off)
        out.append((off, n))
        off += n
    return out


def _split(n, parts):
    out, lo = [], 0
    for p in range(parts):
        hi = (n * (p + 1)) // parts
        out.append(list(range(lo, hi)))
        lo = hi
    return out


def _nt_dot(a, b):
    return jax.lax.dot_general(a, b, (((1,), (1,)), ((), ())),
                               preferred_element_type=jnp.float32)


def _dot(a, b):
    return jnp.dot(a, b, preferred_element_type=jnp.float32)


class _Scope:
    def __init__(self):
        self.cur = None

    def __call__(self, name):
        if not SCOPES:
            return
        if self.cur is not None:
            self.cur.__exit__(None, None, None)
        self.cur = None
        if name is not None:
            self.cur = jax.named_scope(name)
            self.cur.__enter__()


def _kernel(x_hbm, kc_hbm, vc_hbm, awq_hbm, awo_hbm, ckv_hbm, bwq_hbm, wuk_hbm,
            wuv_hbm, bwo_hbm, gw_hbm, o_ref,
            x_v, gw_v, awq_v, awo_v, ckv_v, bwq_v, wuk_v, wuv_v, bwo_v,
            kbuf, vbuf, stack_v, q3_v, acco_v, wsem, ksem, vsem):
    bf16, f32 = jnp.bfloat16, jnp.float32
    scope = _Scope()

    def halves(src, dst, sem, half, lo, n, piece, src_base=0):
        for off, m in _pieces(n, piece):
            for p in range(2):
                r = lo + off + p * half
                pltpu.make_async_copy(src.at[pl.ds(src_base + r, m)], dst.at[pl.ds(r, m)],
                                      sem).start(priority=p)

    kv_pieces = _pieces(_SK, _P256)

    def issue_kv(head, slot, idxs):
        base = head * _SK
        for j in idxs:
            off, n = kv_pieces[j]
            pltpu.make_async_copy(kc_hbm.at[pl.ds(base + off, n)],
                                  kbuf.at[slot, pl.ds(off, n)], ksem.at[slot]).start(priority=0)
            pltpu.make_async_copy(vc_hbm.at[pl.ds(base + off, n)],
                                  vbuf.at[slot, pl.ds(off, n)], vsem.at[slot]).start(priority=1)

    def wait_all(dst, sem):
        pltpu.make_async_copy(dst, dst, sem).wait()

    scope("P0")
    pltpu.make_async_copy(x_hbm, x_v, wsem.at[0]).start()
    pltpu.make_async_copy(gw_hbm, gw_v, wsem.at[1]).start()
    halves(bwq_hbm, bwq_v, wsem.at[2], 8192, 0, 8192, _P256)
    halves(wuk_hbm, wuk_v, wsem.at[3], 8192, 0, 8192, _P256)

    row256 = jax.lax.broadcasted_iota(jnp.int32, (256, 128), 0)
    lane256 = jax.lax.broadcasted_iota(jnp.int32, (256, 128), 1)
    diag256 = (row256 & 31) == (lane256 & 31)
    row128 = jax.lax.broadcasted_iota(jnp.int32, (128, 128), 0)
    lane128 = jax.lax.broadcasted_iota(jnp.int32, (128, 128), 1)

    def expand(cst, w2_ref, issue):
        def body(s, acc):
            issue(s)
            e_s = (row128 == 4 * s + (lane128 >> 5)).astype(bf16)
            y = jnp.where(diag256, _dot(cst, e_s), 0.0).astype(bf16)
            for j in range(4):
                r0 = pl.multiple_of((32 * j + s) * 128, 128)
                acc = acc + _dot(y[64 * j:64 * j + 64], w2_ref[pl.ds(r0, 128), :])
            return acc
        return jax.lax.fori_loop(0, 32, body, jnp.zeros((64, 128), f32))

    def absorb(q, w2_ref, issue):
        def body(s, acc):
            issue(s)
            ts = []
            for j in range(4):
                r0 = pl.multiple_of((32 * j + s) * 128, 128)
                ts.append(_nt_dot(q, w2_ref[pl.ds(r0, 128), :]))
            t = jnp.where(diag256, jnp.concatenate(ts, axis=0), 0.0).astype(bf16)
            g_s = (lane128 == 4 * s + (row128 >> 5)).astype(bf16)
            return acc + _dot(t, g_s)
        return jax.lax.fori_loop(0, 32, body, jnp.zeros((256, 128), f32))

    wait_all(x_v, wsem.at[0])
    row8 = jax.lax.broadcasted_iota(jnp.int32, (8, _DM), 0)
    x0 = x_v[0:1, :].astype(f32)
    x1 = x_v[1:2, :].astype(f32)
    x8 = jnp.where(row8 == 0, jnp.broadcast_to(x0, (8, _DM)),
                   jnp.where(row8 == 1, jnp.broadcast_to(x1, (8, _DM)), 0.0))
    row64 = jax.lax.broadcasted_iota(jnp.int32, (64, 128), 0)
    for j in range(4):
        xa = jnp.broadcast_to(x0[:, 128 * j:128 * j + 128], (64, 128))
        xb = jnp.broadcast_to(x1[:, 128 * j:128 * j + 128], (64, 128))
        stack_v[64 * j:64 * j + 64, :] = jnp.where(row64 < 32, xa, xb).astype(bf16)

    def issue_ckv(b):
        def f(s):
            lo = pl.multiple_of(s * 128, 128)
            halves(ckv_hbm, ckv_v.at[b], wsem.at[4 + b], 4096, lo, 128, _P1K, src_base=b * _SK)
        return f

    scope("B_q")
    wait_all(bwq_v, wsem.at[2])
    q_b = expand(stack_v[...], bwq_v, issue_ckv(0)).astype(bf16)
    scope("B_absorb")
    wait_all(wuk_v, wsem.at[3])
    stack_v[...] = absorb(q_b, wuk_v, issue_ckv(1)).astype(bf16)

    scope("B_attn")
    qa = [jnp.concatenate([stack_v[64 * j + 32 * b:64 * j + 32 * b + 32, :] for j in range(4)], axis=1)
          for b in range(_B)]
    n_t = _SK // _CKV_CHUNK
    for b in range(_B):
        wait_all(ckv_v.at[b], wsem.at[4 + b])

        def bstep(t, carry, b=b):
            m, l, acc = carry
            if b == 0:
                halves(wuv_hbm, wuv_v, wsem.at[6], 8192, pl.multiple_of(t * (8192 // n_t), 16), 8192 // n_t, _P256)
                halves(awq_hbm, awq_v, wsem.at[8], 256, pl.multiple_of(t * (256 // n_t), 16), 256 // n_t, 16)
            else:
                halves(bwo_hbm, bwo_v, wsem.at[7], 2048, pl.multiple_of(t * (2048 // n_t), 16), 2048 // n_t, _P1K)
                halves(awo_hbm, awo_v, wsem.at[9], 2048, pl.multiple_of(t * (2048 // n_t), 16), 2048 // n_t, _P1K)
            c = ckv_v[b, pl.ds(pl.multiple_of(t * _CKV_CHUNK, _CKV_CHUNK), _CKV_CHUNK), :]
            s = _nt_dot(qa[b], c) * _SCALE
            m_new = jnp.maximum(m, jnp.max(s, axis=1, keepdims=True))
            alpha = jnp.exp(m - m_new)
            p = jnp.exp(s - m_new)
            l = alpha * l + jnp.sum(p, axis=1, keepdims=True)
            acc = alpha * acc + _dot(p.astype(bf16), c)
            return m_new, l, acc
        init = (jnp.full((32, 1), -1e30, f32), jnp.zeros((32, 1), f32), jnp.zeros((32, _DC), f32))
        _, l, acc = jax.lax.fori_loop(0, n_t, bstep, init)
        ctx_c = (acc / l).astype(bf16)
        for j in range(4):
            stack_v[64 * j + 32 * b:64 * j + 32 * b + 32, :] = ctx_c[:, 128 * j:128 * j + 128]

    scope("B_uv")
    wait_all(wuv_v, wsem.at[6])

    def issue_first_heads(s):
        head = s // 16
        lo = pl.multiple_of((s % 16) * 512, 512)
        for off, n in _pieces(512, _P256):
            pltpu.make_async_copy(kc_hbm.at[pl.ds(head * _SK + lo + off, n)],
                                  kbuf.at[head, pl.ds(lo + off, n)], ksem.at[head]).start(priority=0)
            pltpu.make_async_copy(vc_hbm.at[pl.ds(head * _SK + lo + off, n)],
                                  vbuf.at[head, pl.ds(lo + off, n)], vsem.at[head]).start(priority=1)
    ctx = expand(stack_v[...], wuv_v, issue_first_heads)

    scope("B_wo")
    wait_all(bwo_v, wsem.at[7])
    row8s = jax.lax.broadcasted_iota(jnp.int32, (8, 128), 0)
    out_b = jnp.zeros((8, _DM), f32)
    groups = _split(len(kv_pieces), _H)
    for h in range(_H):
        for hd in range(2, _AHEAD):
            issue_kv(hd, hd, groups[h])
        lhs = jnp.where(row8s == 0, jnp.broadcast_to(ctx[h:h + 1], (8, 128)),
                        jnp.where(row8s == 1, jnp.broadcast_to(ctx[32 + h:33 + h], (8, 128)), 0.0))
        out_b = out_b + _dot(lhs.astype(bf16), bwo_v[128 * h:128 * h + 128, :])

    scope("A_q")
    wait_all(awq_v, wsem.at[8])
    q_a = _dot(x8.astype(bf16), awq_v[...]).astype(bf16).astype(f32)
    for b in range(_B):
        for h in range(_H):
            q3_v[b * _H + h] = jnp.broadcast_to(q_a[b:b + 1, 128 * h:128 * h + 128], (8, 128))
    acco_v[...] = jnp.zeros(acco_v.shape, f32)
    wait_all(awo_v, wsem.at[9])

    scope("A_loop")
    part = _SK // _NPART
    igroups = _split(len(kv_pieces), 2 * _NPART)

    def head_step(i, carry, do_issue):
        slot = i % _NBUF
        nslot = (i + _AHEAD) % _NBUF
        b = i // _H
        h = i % _H
        q = q3_v[i].astype(bf16)
        pltpu.make_async_copy(kbuf.at[slot], kbuf.at[slot], ksem.at[slot]).wait()
        ss = []
        for c in range(_NPART):
            ss.append(_nt_dot(q, kbuf[slot, c * part:(c + 1) * part, :]))
            if do_issue:
                issue_kv(i + _AHEAD, nslot, igroups[c])
        m = ss[0]
        for c in range(1, _NPART):
            m = jnp.maximum(m, ss[c])
        m = jnp.max(m, axis=1, keepdims=True)
        ps = [jnp.exp2((s - m) * (_SCALE * _LOG2E)) for s in ss]
        l = ps[0]
        for c in range(1, _NPART):
            l = l + ps[c]
        l = jnp.sum(l, axis=1, keepdims=True)
        pltpu.make_async_copy(vbuf.at[slot], vbuf.at[slot], vsem.at[slot]).wait()
        o = None
        for c in range(_NPART):
            oc = _dot(ps[c].astype(bf16), vbuf[slot, c * part:(c + 1) * part, :])
            o = oc if o is None else o + oc
            if do_issue:
                issue_kv(i + _AHEAD, nslot, igroups[_NPART + c])
        o = o / l
        wo = awo_v[pl.ds(pl.multiple_of(h * 128, 128), 128), :]
        acco_v[b] = acco_v[b] + _dot(o.astype(bf16), wo)
        return carry
    jax.lax.fori_loop(0, _NBH - _AHEAD, lambda i, c: head_step(i, c, True), 0)
    scope("A_tail")
    jax.lax.fori_loop(_NBH - _AHEAD, _NBH, lambda i, c: head_step(i, c, False), 0)

    scope("mix")
    wait_all(gw_v, wsem.at[1])
    gw = gw_v[...].astype(f32).reshape(1, _DM)
    g = jax.nn.sigmoid(jnp.sum(x8 * gw, axis=1, keepdims=True))
    for b in range(_B):
        gb = g[b:b + 1]
        res = gb * acco_v[b, 0:1, :] + (1.0 - gb) * out_b[b:b + 1]
        o_ref[b:b + 1, :] = res.astype(o_ref.dtype)
    scope(None)


@jax.jit
def pallas_gated_mix__mha_block_cached__compressed_kv_cla__decode_kernel(
    A_x, A_k_cache, A_v_cache, A_wq, A_wo, B_x, B_c_kv, B_w_q, B_w_uk, B_w_uv, B_w_o, gate_w,
):
    del B_x
    bf16, f32 = jnp.bfloat16, jnp.float32
    kc = A_k_cache.reshape(_NBH * _SK, _DH)
    vc = A_v_cache.reshape(_NBH * _SK, _DH)
    ckv = B_c_kv.reshape(_B * _SK, _DC)
    bwq = B_w_q.reshape(_DM * _H, _DH)
    wuk = B_w_uk.reshape(_DC * _H, _DH)
    wuv = B_w_uv.reshape(_DC * _H, _DH)
    bwo = B_w_o.reshape(_H * _DH, _DM)

    any_spec = pl.BlockSpec(memory_space=pl.ANY)
    scratch = [
        pltpu.VMEM((_B, _DM), bf16),
        pltpu.VMEM((_DM,), bf16),
        pltpu.VMEM((_DM, _H * _DH), bf16),
        pltpu.VMEM((_H * _DH, _DM), bf16),
        pltpu.VMEM((_B, _SK, _DC), bf16),
        pltpu.VMEM((_DM * _H, _DH), bf16),
        pltpu.VMEM((_DC * _H, _DH), bf16),
        pltpu.VMEM((_DC * _H, _DH), bf16),
        pltpu.VMEM((_H * _DH, _DM), bf16),
        pltpu.VMEM((_NBUF, _SK, _DH), bf16),
        pltpu.VMEM((_NBUF, _SK, _DH), bf16),
        pltpu.VMEM((256, 128), bf16),
        pltpu.VMEM((_NBH, 8, _DH), f32),
        pltpu.VMEM((_B, 8, _DM), f32),
        pltpu.SemaphoreType.DMA((10,)),
        pltpu.SemaphoreType.DMA((_NBUF,)),
        pltpu.SemaphoreType.DMA((_NBUF,)),
    ]
    out = pl.pallas_call(
        _kernel,
        out_shape=jax.ShapeDtypeStruct((_B, _DM), bf16),
        in_specs=[any_spec] * 11,
        out_specs=pl.BlockSpec(memory_space=pltpu.VMEM),
        scratch_shapes=scratch,
        compiler_params=pltpu.CompilerParams(vmem_limit_bytes=100 * 1024 * 1024),
    )(A_x.reshape(_B, _DM), kc, vc, A_wq, A_wo, ckv, bwq, wuk, wuv, bwo, gate_w)
    return out.reshape(_B, 1, _DM)
```

```python
import jax
import jax.numpy as jnp
import jax.experimental.pallas as pl
import jax.experimental.pallas.tpu as pltpu

_B, _H, _SK, _DH, _DM, _DC = 2, 32, 8192, 128, 512, 512
_NBH = _B * _H
_LOG2E = 1.4426950408889634
_SCALE = _DH ** -0.5

_NBUF = 4
_AHEAD = 3
_P256 = 192
_P1K = 48
_CKV_CHUNK = 1024
_NPART = 4
SCOPES = False
U32 = True
BEND = 1
PLAN = [0, 0, 0, 0, 0, 0, 0, 0, 0, 1]
def _wsplit(n, weights):
    tot = sum(weights); out = []; lo = 0; acc = 0
    for w in weights:
        acc += w
        hi = (n * acc) // tot
        out.append(list(range(lo, hi))); lo = hi
    return out


def _pieces(total, piece):
    out, off = [], 0
    while off < total:
        n = min(piece, total - off)
        out.append((off, n))
        off += n
    return out


def _split(n, parts):
    out, lo = [], 0
    for p in range(parts):
        hi = (n * (p + 1)) // parts
        out.append(list(range(lo, hi)))
        lo = hi
    return out


def _nt_dot(a, b):
    return jax.lax.dot_general(a, b, (((1,), (1,)), ((), ())),
                               preferred_element_type=jnp.float32)


def _dot(a, b):
    return jnp.dot(a, b, preferred_element_type=jnp.float32)


class _Scope:
    def __init__(self):
        self.cur = None

    def __call__(self, name):
        if not SCOPES:
            return
        if self.cur is not None:
            self.cur.__exit__(None, None, None)
        self.cur = None
        if name is not None:
            self.cur = jax.named_scope(name)
            self.cur.__enter__()


def _kernel(x_hbm, kc_hbm, vc_hbm, awq_hbm, awo_hbm, ckv_hbm, bwq_hbm, wuk_hbm,
            wuv_hbm, bwo_hbm, gw_hbm, o_ref,
            x_v, gw_v, awq_v, awo_v, ckv_v, bwq_v, wuk_v, wuv_v, bwo_v,
            kbuf, vbuf, stack_v, q3_v, acco_v, wsem, ksem, vsem):
    bf16, f32 = jnp.bfloat16, jnp.float32
    scope = _Scope()

    def halves(src, dst, sem, half, lo, n, piece, src_base=0):
        for off, m in _pieces(n, piece):
            for p in range(2):
                r = lo + off + p * half
                pltpu.make_async_copy(src.at[pl.ds(src_base + r, m)], dst.at[pl.ds(r, m)],
                                      sem).start(priority=p)

    kv_pieces = _pieces(_SK, _P256)

    def issue_kv(head, slot, idxs):
        base = head * _SK
        for j in idxs:
            off, n = kv_pieces[j]
            pltpu.make_async_copy(kc_hbm.at[pl.ds(base + off, n)],
                                  kbuf.at[slot, pl.ds(off, n)], ksem.at[slot]).start(priority=0)
            pltpu.make_async_copy(vc_hbm.at[pl.ds(base + off, n)],
                                  vbuf.at[slot, pl.ds(off, n)], vsem.at[slot]).start(priority=1)

    def wait_all(dst, sem):
        pltpu.make_async_copy(dst, dst, sem).wait()

    scope("P0")
    pltpu.make_async_copy(x_hbm, x_v, wsem.at[0]).start()
    pltpu.make_async_copy(gw_hbm, gw_v, wsem.at[1]).start()
    halves(bwq_hbm, bwq_v, wsem.at[2], 8192, 0, 8192, _P256)
    halves(wuk_hbm, wuk_v, wsem.at[3], 8192, 0, 8192, _P256)

    row256 = jax.lax.broadcasted_iota(jnp.int32, (256, 128), 0)
    lane256 = jax.lax.broadcasted_iota(jnp.int32, (256, 128), 1)
    diag256 = (row256 & 31) == (lane256 & 31)
    row128 = jax.lax.broadcasted_iota(jnp.int32, (128, 128), 0)
    lane128 = jax.lax.broadcasted_iota(jnp.int32, (128, 128), 1)

    def expand(cst, w2_ref, issue):
        def body(s, acc):
            if not BEND:
                issue(s)
            e_s = (row128 == 4 * s + (lane128 >> 5)).astype(bf16)
            y = jnp.where(diag256, _dot(cst, e_s), 0.0).astype(bf16)
            for j in range(4):
                r0 = pl.multiple_of((32 * j + s) * 128, 128)
                acc = acc + _dot(y[64 * j:64 * j + 64], w2_ref[pl.ds(r0, 128), :])
            if BEND:
                issue(s)
            return acc
        return jax.lax.fori_loop(0, 32, body, jnp.zeros((64, 128), f32))

    def absorb(q, w2_ref, issue):
        def body(s, acc):
            if not BEND:
                issue(s)
            ts = []
            for j in range(4):
                r0 = pl.multiple_of((32 * j + s) * 128, 128)
                ts.append(_nt_dot(q, w2_ref[pl.ds(r0, 128), :]))
            t = jnp.where(diag256, jnp.concatenate(ts, axis=0), 0.0).astype(bf16)
            g_s = (lane128 == 4 * s + (row128 >> 5)).astype(bf16)
            acc = acc + _dot(t, g_s)
            if BEND:
                issue(s)
            return acc
        return jax.lax.fori_loop(0, 32, body, jnp.zeros((256, 128), f32))

    wait_all(x_v, wsem.at[0])
    row8 = jax.lax.broadcasted_iota(jnp.int32, (8, _DM), 0)
    x0 = x_v[0:1, :].astype(f32)
    x1 = x_v[1:2, :].astype(f32)
    x8 = jnp.where(row8 == 0, jnp.broadcast_to(x0, (8, _DM)),
                   jnp.where(row8 == 1, jnp.broadcast_to(x1, (8, _DM)), 0.0))
    row64 = jax.lax.broadcasted_iota(jnp.int32, (64, 128), 0)
    for j in range(4):
        xa = jnp.broadcast_to(x0[:, 128 * j:128 * j + 128], (64, 128))
        xb = jnp.broadcast_to(x1[:, 128 * j:128 * j + 128], (64, 128))
        stack_v[64 * j:64 * j + 64, :] = jnp.where(row64 < 32, xa, xb).astype(bf16)

    def issue_ckv(b):
        def f(s):
            lo = pl.multiple_of(s * 128, 128)
            halves(ckv_hbm, ckv_v.at[b], wsem.at[4 + b], 4096, lo, 128, _P1K, src_base=b * _SK)
        return f

    scope("B_q")
    wait_all(bwq_v, wsem.at[2])
    q_b = expand(stack_v[...], bwq_v, issue_ckv(0)).astype(bf16)
    scope("B_absorb")
    wait_all(wuk_v, wsem.at[3])
    stack_v[...] = absorb(q_b, wuk_v, issue_ckv(1)).astype(bf16)

    scope("B_attn")
    qa = [jnp.concatenate([stack_v[64 * j + 32 * b:64 * j + 32 * b + 32, :] for j in range(4)], axis=1)
          for b in range(_B)]
    n_t = _SK // _CKV_CHUNK
    for b in range(_B):
        wait_all(ckv_v.at[b], wsem.at[4 + b])

        def bstep(t, carry, b=b):
            m, l, acc = carry
            def iss():
              if b == 0:
                halves(wuv_hbm, wuv_v, wsem.at[6], 8192, pl.multiple_of(t * (8192 // n_t), 16), 8192 // n_t, _P256)
                halves(awq_hbm, awq_v, wsem.at[8], 256, pl.multiple_of(t * (256 // n_t), 16), 256 // n_t, 16)
              else:
                halves(bwo_hbm, bwo_v, wsem.at[7], 2048, pl.multiple_of(t * (2048 // n_t), 16), 2048 // n_t, _P1K)
                halves(awo_hbm, awo_v, wsem.at[9], 2048, pl.multiple_of(t * (2048 // n_t), 16), 2048 // n_t, _P1K)
            if not BEND:
                iss()
            c = ckv_v[b, pl.ds(pl.multiple_of(t * _CKV_CHUNK, _CKV_CHUNK), _CKV_CHUNK), :]
            s = _nt_dot(qa[b], c) * _SCALE
            m_new = jnp.maximum(m, jnp.max(s, axis=1, keepdims=True))
            alpha = jnp.exp(m - m_new)
            p = jnp.exp(s - m_new)
            l = alpha * l + jnp.sum(p, axis=1, keepdims=True)
            acc = alpha * acc + _dot(p.astype(bf16), c)
            if BEND:
                iss()
            return m_new, l, acc
        init = (jnp.full((32, 1), -1e30, f32), jnp.zeros((32, 1), f32), jnp.zeros((32, _DC), f32))
        _, l, acc = jax.lax.fori_loop(0, n_t, bstep, init)
        ctx_c = (acc / l).astype(bf16)
        for j in range(4):
            stack_v[64 * j + 32 * b:64 * j + 32 * b + 32, :] = ctx_c[:, 128 * j:128 * j + 128]

    scope("B_uv")
    wait_all(wuv_v, wsem.at[6])

    def issue_first_heads(s):
        head = s // 16
        lo = pl.multiple_of((s % 16) * 512, 512)
        for off, n in _pieces(512, _P256):
            pltpu.make_async_copy(kc_hbm.at[pl.ds(head * _SK + lo + off, n)],
                                  kbuf.at[head, pl.ds(lo + off, n)], ksem.at[head]).start(priority=0)
            pltpu.make_async_copy(vc_hbm.at[pl.ds(head * _SK + lo + off, n)],
                                  vbuf.at[head, pl.ds(lo + off, n)], vsem.at[head]).start(priority=1)
    ctx = expand(stack_v[...], wuv_v, issue_first_heads)

    scope("B_wo")
    wait_all(bwo_v, wsem.at[7])
    row8s = jax.lax.broadcasted_iota(jnp.int32, (8, 128), 0)
    out_b = jnp.zeros((8, _DM), f32)
    groups = _split(len(kv_pieces), _H)
    for h in range(_H):
        for hd in range(2, _AHEAD):
            issue_kv(hd, hd, groups[h])
        lhs = jnp.where(row8s == 0, jnp.broadcast_to(ctx[h:h + 1], (8, 128)),
                        jnp.where(row8s == 1, jnp.broadcast_to(ctx[32 + h:33 + h], (8, 128)), 0.0))
        out_b = out_b + _dot(lhs.astype(bf16), bwo_v[128 * h:128 * h + 128, :])

    scope("A_q")
    wait_all(awq_v, wsem.at[8])
    q_a = _dot(x8.astype(bf16), awq_v[...]).astype(bf16).astype(f32)
    for b in range(_B):
        for h in range(_H):
            q3_v[b * _H + h] = jnp.broadcast_to(q_a[b:b + 1, 128 * h:128 * h + 128], (8, 128))
    acco_v[...] = jnp.zeros(acco_v.shape, f32)
    wait_all(awo_v, wsem.at[9])

    scope("A_loop")
    kbuf32 = kbuf.bitcast(jnp.uint32)
    vbuf32 = vbuf.bitcast(jnp.uint32)

    def ldk(buf, buf32, slot, c):
        if U32:
            return pltpu.bitcast(buf32[slot, c * (part // 2):(c + 1) * (part // 2), :], bf16)
        return buf[slot, c * part:(c + 1) * part, :]
    part = _SK // _NPART
    igroups = _wsplit(len(kv_pieces), PLAN)
    assert len(PLAN) == 2 * _NPART + 2

    def head_step(i, carry, do_issue):
        slot = i % _NBUF
        nslot = (i + _AHEAD) % _NBUF
        b = i // _H
        h = i % _H
        q = q3_v[i].astype(bf16)
        pltpu.make_async_copy(kbuf.at[slot], kbuf.at[slot], ksem.at[slot]).wait()
        ss = []
        if do_issue:
            issue_kv(i + _AHEAD, nslot, igroups[0])
        for c in range(_NPART):
            ss.append(_nt_dot(q, ldk(kbuf, kbuf32, slot, c)))
            if do_issue:
                issue_kv(i + _AHEAD, nslot, igroups[1 + c])
        m = ss[0]
        for c in range(1, _NPART):
            m = jnp.maximum(m, ss[c])
        m = jnp.max(m, axis=1, keepdims=True)
        ps = [jnp.exp2((s - m) * (_SCALE * _LOG2E)) for s in ss]
        l = ps[0]
        for c in range(1, _NPART):
            l = l + ps[c]
        l = jnp.sum(l, axis=1, keepdims=True)
        pltpu.make_async_copy(vbuf.at[slot], vbuf.at[slot], vsem.at[slot]).wait()
        o = None
        if do_issue:
            issue_kv(i + _AHEAD, nslot, igroups[_NPART + 1])
        for c in range(_NPART):
            oc = _dot(ps[c].astype(bf16), ldk(vbuf, vbuf32, slot, c))
            o = oc if o is None else o + oc
            if do_issue:
                issue_kv(i + _AHEAD, nslot, igroups[_NPART + 2 + c])
        o = o / l
        wo = awo_v[pl.ds(pl.multiple_of(h * 128, 128), 128), :]
        acco_v[b] = acco_v[b] + _dot(o.astype(bf16), wo)
        return carry
    jax.lax.fori_loop(0, _NBH - _AHEAD, lambda i, c: head_step(i, c, True), 0)
    scope("A_tail")
    jax.lax.fori_loop(_NBH - _AHEAD, _NBH, lambda i, c: head_step(i, c, False), 0)

    scope("mix")
    wait_all(gw_v, wsem.at[1])
    gw = gw_v[...].astype(f32).reshape(1, _DM)
    g = jax.nn.sigmoid(jnp.sum(x8 * gw, axis=1, keepdims=True))
    for b in range(_B):
        gb = g[b:b + 1]
        res = gb * acco_v[b, 0:1, :] + (1.0 - gb) * out_b[b:b + 1]
        o_ref[b:b + 1, :] = res.astype(o_ref.dtype)
    scope(None)


@jax.jit
def pallas_gated_mix__mha_block_cached__compressed_kv_cla__decode_kernel(
    A_x, A_k_cache, A_v_cache, A_wq, A_wo, B_x, B_c_kv, B_w_q, B_w_uk, B_w_uv, B_w_o, gate_w,
):
    del B_x
    bf16, f32 = jnp.bfloat16, jnp.float32
    kc = A_k_cache.reshape(_NBH * _SK, _DH)
    vc = A_v_cache.reshape(_NBH * _SK, _DH)
    ckv = B_c_kv.reshape(_B * _SK, _DC)
    bwq = B_w_q.reshape(_DM * _H, _DH)
    wuk = B_w_uk.reshape(_DC * _H, _DH)
    wuv = B_w_uv.reshape(_DC * _H, _DH)
    bwo = B_w_o.reshape(_H * _DH, _DM)

    any_spec = pl.BlockSpec(memory_space=pl.ANY)
    scratch = [
        pltpu.VMEM((_B, _DM), bf16),
        pltpu.VMEM((_DM,), bf16),
        pltpu.VMEM((_DM, _H * _DH), bf16),
        pltpu.VMEM((_H * _DH, _DM), bf16),
        pltpu.VMEM((_B, _SK, _DC), bf16),
        pltpu.VMEM((_DM * _H, _DH), bf16),
        pltpu.VMEM((_DC * _H, _DH), bf16),
        pltpu.VMEM((_DC * _H, _DH), bf16),
        pltpu.VMEM((_H * _DH, _DM), bf16),
        pltpu.VMEM((_NBUF, _SK, _DH), bf16),
        pltpu.VMEM((_NBUF, _SK, _DH), bf16),
        pltpu.VMEM((256, 128), bf16),
        pltpu.VMEM((_NBH, 8, _DH), f32),
        pltpu.VMEM((_B, 8, _DM), f32),
        pltpu.SemaphoreType.DMA((10,)),
        pltpu.SemaphoreType.DMA((_NBUF,)),
        pltpu.SemaphoreType.DMA((_NBUF,)),
    ]
    out = pl.pallas_call(
        _kernel,
        out_shape=jax.ShapeDtypeStruct((_B, _DM), bf16),
        in_specs=[any_spec] * 11,
        out_specs=pl.BlockSpec(memory_space=pltpu.VMEM),
        scratch_shapes=scratch,
        compiler_params=pltpu.CompilerParams(vmem_limit_bytes=100 * 1024 * 1024),
    )(A_x.reshape(_B, _DM), kc, vc, A_wq, A_wo, ckv, bwq, wuk, wuv, bwo, gate_w)
    return out.reshape(_B, 1, _DM)
```

```python
import jax
import jax.numpy as jnp
import jax.experimental.pallas as pl
import jax.experimental.pallas.tpu as pltpu

_B, _H, _SK, _DH, _DM, _DC = 2, 32, 8192, 128, 512, 512
_NBH = _B * _H
_SCALE = _DH ** -0.5
_LOG2E = 1.4426950408889634

_NBUF = 4
_AHEAD = 3
_P256 = 192
_P1K = 48
_CKV_CHUNK = 1024


def _pieces(total, piece):
    out, off = [], 0
    while off < total:
        n = min(piece, total - off)
        out.append((off, n))
        off += n
    return out


def _split(n, parts):
    bounds = [(n * p) // parts for p in range(parts + 1)]
    return [list(range(bounds[p], bounds[p + 1])) for p in range(parts)]


def _nt_dot(a, b):
    return jax.lax.dot_general(a, b, (((1,), (1,)), ((), ())),
                               preferred_element_type=jnp.float32)


def _dot(a, b):
    return jnp.dot(a, b, preferred_element_type=jnp.float32)


def _kernel(x_hbm, kc_hbm, vc_hbm, awq_hbm, awo_hbm, ckv_hbm, bwq_hbm, wuk_hbm,
            wuv_hbm, bwo_hbm, gw_hbm, o_ref,
            x_v, gw_v, awq_v, awo_v, ckv_v, bwq_v, wuk_v, wuv_v, bwo_v,
            kbuf, vbuf, stack_v, q3_v, acco_v, wsem, ksem, vsem):
    bf16, f32 = jnp.bfloat16, jnp.float32

    def halves(src, dst, sem, half, lo, n, piece, src_base=0):
        for off, m in _pieces(n, piece):
            for p in range(2):
                r = lo + off + p * half
                pltpu.make_async_copy(src.at[pl.ds(src_base + r, m)], dst.at[pl.ds(r, m)],
                                      sem).start(priority=p)

    kv_pieces = _pieces(_SK, _P256)

    def issue_kv(head, slot, idxs):
        base = head * _SK
        for j in idxs:
            off, n = kv_pieces[j]
            pltpu.make_async_copy(kc_hbm.at[pl.ds(base + off, n)],
                                  kbuf.at[slot, pl.ds(off, n)], ksem.at[slot]).start(priority=0)
            pltpu.make_async_copy(vc_hbm.at[pl.ds(base + off, n)],
                                  vbuf.at[slot, pl.ds(off, n)], vsem.at[slot]).start(priority=1)

    def wait_all(dst, sem):
        pltpu.make_async_copy(dst, dst, sem).wait()

    row256 = jax.lax.broadcasted_iota(jnp.int32, (256, 128), 0)
    lane256 = jax.lax.broadcasted_iota(jnp.int32, (256, 128), 1)
    diag256 = (row256 & 31) == (lane256 & 31)
    row128 = jax.lax.broadcasted_iota(jnp.int32, (128, 128), 0)
    lane128 = jax.lax.broadcasted_iota(jnp.int32, (128, 128), 1)

    def expand(cst, w2_ref, issue):
        def body(s, acc):
            e_s = (row128 == 4 * s + (lane128 >> 5)).astype(bf16)
            y = jnp.where(diag256, _dot(cst, e_s), 0.0).astype(bf16)
            for j in range(4):
                r0 = pl.multiple_of((32 * j + s) * 128, 128)
                acc = acc + _dot(y[64 * j:64 * j + 64], w2_ref[pl.ds(r0, 128), :])
            issue(s)
            return acc
        return jax.lax.fori_loop(0, 32, body, jnp.zeros((64, 128), f32))

    def absorb(q, w2_ref, issue):
        def body(s, acc):
            ts = []
            for j in range(4):
                r0 = pl.multiple_of((32 * j + s) * 128, 128)
                ts.append(_nt_dot(q, w2_ref[pl.ds(r0, 128), :]))
            t = jnp.where(diag256, jnp.concatenate(ts, axis=0), 0.0).astype(bf16)
            g_s = (lane128 == 4 * s + (row128 >> 5)).astype(bf16)
            acc = acc + _dot(t, g_s)
            issue(s)
            return acc
        return jax.lax.fori_loop(0, 32, body, jnp.zeros((256, 128), f32))

    pltpu.make_async_copy(x_hbm, x_v, wsem.at[0]).start()
    pltpu.make_async_copy(gw_hbm, gw_v, wsem.at[1]).start()
    halves(bwq_hbm, bwq_v, wsem.at[2], 8192, 0, 8192, _P256)
    halves(wuk_hbm, wuk_v, wsem.at[3], 8192, 0, 8192, _P256)

    wait_all(x_v, wsem.at[0])
    row8 = jax.lax.broadcasted_iota(jnp.int32, (8, _DM), 0)
    x0 = x_v[0:1, :].astype(f32)
    x1 = x_v[1:2, :].astype(f32)
    x8 = jnp.where(row8 == 0, jnp.broadcast_to(x0, (8, _DM)),
                   jnp.where(row8 == 1, jnp.broadcast_to(x1, (8, _DM)), 0.0))
    row64 = jax.lax.broadcasted_iota(jnp.int32, (64, 128), 0)
    for j in range(4):
        xa = jnp.broadcast_to(x0[:, 128 * j:128 * j + 128], (64, 128))
        xb = jnp.broadcast_to(x1[:, 128 * j:128 * j + 128], (64, 128))
        stack_v[64 * j:64 * j + 64, :] = jnp.where(row64 < 32, xa, xb).astype(bf16)

    def issue_ckv(b):
        def f(s):
            lo = pl.multiple_of(s * 128, 128)
            halves(ckv_hbm, ckv_v.at[b], wsem.at[4 + b], _SK // 2, lo, 128, _P1K, src_base=b * _SK)
        return f

    wait_all(bwq_v, wsem.at[2])
    q_b = expand(stack_v[...], bwq_v, issue_ckv(0)).astype(bf16)
    wait_all(wuk_v, wsem.at[3])
    stack_v[...] = absorb(q_b, wuk_v, issue_ckv(1)).astype(bf16)

    qa = [jnp.concatenate([stack_v[64 * j + 32 * b:64 * j + 32 * b + 32, :] for j in range(4)], axis=1)
          for b in range(_B)]
    n_t = _SK // _CKV_CHUNK
    for b in range(_B):
        wait_all(ckv_v.at[b], wsem.at[4 + b])

        def bstep(t, carry, b=b):
            m, l, acc = carry
            c = ckv_v[b, pl.ds(pl.multiple_of(t * _CKV_CHUNK, _CKV_CHUNK), _CKV_CHUNK), :]
            s = _nt_dot(qa[b], c) * _SCALE
            m_new = jnp.maximum(m, jnp.max(s, axis=1, keepdims=True))
            alpha = jnp.exp(m - m_new)
            p = jnp.exp(s - m_new)
            l = alpha * l + jnp.sum(p, axis=1, keepdims=True)
            acc = alpha * acc + _dot(p.astype(bf16), c)
            if b == 0:
                halves(wuv_hbm, wuv_v, wsem.at[6], 8192,
                       pl.multiple_of(t * (8192 // n_t), 16), 8192 // n_t, _P256)
                halves(awq_hbm, awq_v, wsem.at[8], 256,
                       pl.multiple_of(t * (256 // n_t), 16), 256 // n_t, 16)
            else:
                halves(bwo_hbm, bwo_v, wsem.at[7], 2048,
                       pl.multiple_of(t * (2048 // n_t), 16), 2048 // n_t, _P1K)
                halves(awo_hbm, awo_v, wsem.at[9], 2048,
                       pl.multiple_of(t * (2048 // n_t), 16), 2048 // n_t, _P1K)
            return m_new, l, acc
        init = (jnp.full((32, 1), -1e30, f32), jnp.zeros((32, 1), f32), jnp.zeros((32, _DC), f32))
        _, l, acc = jax.lax.fori_loop(0, n_t, bstep, init)
        ctx_c = (acc / l).astype(bf16)
        for j in range(4):
            stack_v[64 * j + 32 * b:64 * j + 32 * b + 32, :] = ctx_c[:, 128 * j:128 * j + 128]

    def issue_first_heads(s):
        head = s // 16
        lo = pl.multiple_of((s % 16) * 512, 512)
        for off, n in _pieces(512, _P256):
            pltpu.make_async_copy(kc_hbm.at[pl.ds(head * _SK + lo + off, n)],
                                  kbuf.at[head, pl.ds(lo + off, n)], ksem.at[head]).start(priority=0)
            pltpu.make_async_copy(vc_hbm.at[pl.ds(head * _SK + lo + off, n)],
                                  vbuf.at[head, pl.ds(lo + off, n)], vsem.at[head]).start(priority=1)

    wait_all(wuv_v, wsem.at[6])
    ctx = expand(stack_v[...], wuv_v, issue_first_heads)

    wait_all(bwo_v, wsem.at[7])
    row8s = jax.lax.broadcasted_iota(jnp.int32, (8, 128), 0)
    out_b = jnp.zeros((8, _DM), f32)
    groups = _split(len(kv_pieces), _H)
    for h in range(_H):
        for hd in range(2, _AHEAD):
            issue_kv(hd, hd, groups[h])
        lhs = jnp.where(row8s == 0, jnp.broadcast_to(ctx[h:h + 1], (8, 128)),
                        jnp.where(row8s == 1, jnp.broadcast_to(ctx[32 + h:33 + h], (8, 128)), 0.0))
        out_b = out_b + _dot(lhs.astype(bf16), bwo_v[128 * h:128 * h + 128, :])

    wait_all(awq_v, wsem.at[8])
    q_a = _dot(x8.astype(bf16), awq_v[...]).astype(bf16).astype(f32)
    for b in range(_B):
        for h in range(_H):
            q3_v[b * _H + h] = jnp.broadcast_to(q_a[b:b + 1, 128 * h:128 * h + 128], (8, 128))
    acco_v[...] = jnp.zeros(acco_v.shape, f32)
    wait_all(awo_v, wsem.at[9])

    def head_step(i, carry, do_issue):
        slot = i % _NBUF
        b = i // _H
        h = i % _H
        q = q3_v[i].astype(bf16)
        wait_all(kbuf.at[slot], ksem.at[slot])
        s = _nt_dot(q, kbuf[slot])
        m = jnp.max(s, axis=1, keepdims=True)
        p = jnp.exp2((s - m) * (_SCALE * _LOG2E))
        l = jnp.sum(p, axis=1, keepdims=True)
        wait_all(vbuf.at[slot], vsem.at[slot])
        o = _dot(p.astype(bf16), vbuf[slot]) / l
        if do_issue:
            issue_kv(i + _AHEAD, (i + _AHEAD) % _NBUF, range(len(kv_pieces)))
        wo = awo_v[pl.ds(pl.multiple_of(h * 128, 128), 128), :]
        acco_v[b] = acco_v[b] + _dot(o.astype(bf16), wo)
        return carry
    jax.lax.fori_loop(0, _NBH - _AHEAD, lambda i, c: head_step(i, c, True), 0)
    jax.lax.fori_loop(_NBH - _AHEAD, _NBH, lambda i, c: head_step(i, c, False), 0)

    wait_all(gw_v, wsem.at[1])
    gw = gw_v[...].astype(f32).reshape(1, _DM)
    g = jax.nn.sigmoid(jnp.sum(x8 * gw, axis=1, keepdims=True))
    out_a = jnp.where(row8 == 0, acco_v[0], acco_v[1])
    res = g * out_a + (1.0 - g) * out_b
    o_ref[...] = res[0:_B, :].astype(o_ref.dtype)


@jax.jit
def pallas_gated_mix__mha_block_cached__compressed_kv_cla__decode_kernel(
    A_x: jax.Array,
    A_k_cache: jax.Array,
    A_v_cache: jax.Array,
    A_wq: jax.Array,
    A_wo: jax.Array,
    B_x: jax.Array,
    B_c_kv: jax.Array,
    B_w_q: jax.Array,
    B_w_uk: jax.Array,
    B_w_uv: jax.Array,
    B_w_o: jax.Array,
    gate_w: jax.Array,
):
    del B_x
    bf16, f32 = jnp.bfloat16, jnp.float32
    x = A_x.reshape(_B, _DM)
    kc = A_k_cache.reshape(_NBH * _SK, _DH)
    vc = A_v_cache.reshape(_NBH * _SK, _DH)
    ckv = B_c_kv.reshape(_B * _SK, _DC)
    bwq = B_w_q.reshape(_DM * _H, _DH)
    wuk = B_w_uk.reshape(_DC * _H, _DH)
    wuv = B_w_uv.reshape(_DC * _H, _DH)
    bwo = B_w_o.reshape(_H * _DH, _DM)

    scratch = [
        pltpu.VMEM((_B, _DM), bf16),
        pltpu.VMEM((_DM,), bf16),
        pltpu.VMEM((_DM, _H * _DH), bf16),
        pltpu.VMEM((_H * _DH, _DM), bf16),
        pltpu.VMEM((_B, _SK, _DC), bf16),
        pltpu.VMEM((_DM * _H, _DH), bf16),
        pltpu.VMEM((_DC * _H, _DH), bf16),
        pltpu.VMEM((_DC * _H, _DH), bf16),
        pltpu.VMEM((_H * _DH, _DM), bf16),
        pltpu.VMEM((_NBUF, _SK, _DH), bf16),
        pltpu.VMEM((_NBUF, _SK, _DH), bf16),
        pltpu.VMEM((256, 128), bf16),
        pltpu.VMEM((_NBH, 8, _DH), f32),
        pltpu.VMEM((_B, 8, _DM), f32),
        pltpu.SemaphoreType.DMA((10,)),
        pltpu.SemaphoreType.DMA((_NBUF,)),
        pltpu.SemaphoreType.DMA((_NBUF,)),
    ]
    out = pl.pallas_call(
        _kernel,
        out_shape=jax.ShapeDtypeStruct((_B, _DM), bf16),
        in_specs=[pl.BlockSpec(memory_space=pl.ANY)] * 11,
        out_specs=pl.BlockSpec(memory_space=pltpu.VMEM),
        scratch_shapes=scratch,
        compiler_params=pltpu.CompilerParams(vmem_limit_bytes=100 * 1024 * 1024),
    )(x, kc, vc, A_wq, A_wo, ckv, bwq, wuk, wuv, bwo, gate_w)
    return out.reshape(_B, 1, _DM)
```

```python
import jax
import jax.numpy as jnp
import jax.experimental.pallas as pl
import jax.experimental.pallas.tpu as pltpu

_B, _H, _SK, _DH, _DM, _DC = 2, 32, 8192, 128, 512, 512
_NBH = _B * _H
_SCALE = _DH ** -0.5
_LOG2E = 1.4426950408889634

_NBUF = 4
_AHEAD = 3
_P256 = 192
_P1K = 48
_CKV_CHUNK = 1024


def _pieces(total, piece):
    out, off = [], 0
    while off < total:
        n = min(piece, total - off)
        out.append((off, n))
        off += n
    return out


def _even_pieces(total, piece, align):
    n = -(-total // piece)
    units = total // align
    bounds = [(units * k) // n * align for k in range(n + 1)]
    return [(bounds[k], bounds[k + 1] - bounds[k]) for k in range(n)]


def _nt_dot(a, b):
    return jax.lax.dot_general(a, b, (((1,), (1,)), ((), ())),
                               preferred_element_type=jnp.float32)


def _dot(a, b):
    return jnp.dot(a, b, preferred_element_type=jnp.float32)


def _kernel(x_hbm, kc_hbm, vc_hbm, awq_hbm, awo_hbm, ckv_hbm, bwq_hbm, wuk_hbm,
            wuv_hbm, bwo_hbm, gw_hbm, o_hbm,
            x_v, gw_v, awq_v, awo_v, ckv_v, bwq_v, wuk_v, wuv_v, bwo_v,
            kbuf, vbuf, stack_v, q3_v, acco_v, out_v, wsem, ksem, vsem, osem):
    bf16, f32 = jnp.bfloat16, jnp.float32

    def halves(src, dst, sem, half, lo, pieces, src_base=0):
        for off, m in pieces:
            for p in range(2):
                r = lo + off + p * half
                pltpu.make_async_copy(src.at[pl.ds(src_base + r, m)], dst.at[pl.ds(r, m)],
                                      sem).start(priority=p)

    kv_pieces = _pieces(_SK, _P256)

    def issue_kv(head, slot, idxs):
        base = head * _SK
        for j in idxs:
            off, n = kv_pieces[j]
            pltpu.make_async_copy(kc_hbm.at[pl.ds(base + off, n)],
                                  kbuf.at[slot, pl.ds(off, n)], ksem.at[slot]).start(priority=0)
            pltpu.make_async_copy(vc_hbm.at[pl.ds(base + off, n)],
                                  vbuf.at[slot, pl.ds(off, n)], vsem.at[slot]).start(priority=1)

    def wait_all(dst, sem):
        pltpu.make_async_copy(dst, dst, sem).wait()

    row256 = jax.lax.broadcasted_iota(jnp.int32, (256, 128), 0)
    lane256 = jax.lax.broadcasted_iota(jnp.int32, (256, 128), 1)
    diag256 = (row256 & 31) == (lane256 & 31)
    row128 = jax.lax.broadcasted_iota(jnp.int32, (128, 128), 0)
    lane128 = jax.lax.broadcasted_iota(jnp.int32, (128, 128), 1)

    def expand(cst, w2_ref, issue):
        def body(s, acc):
            e_s = (row128 == 4 * s + (lane128 >> 5)).astype(bf16)
            y = jnp.where(diag256, _dot(cst, e_s), 0.0).astype(bf16)
            for j in range(4):
                r0 = pl.multiple_of((32 * j + s) * 128, 128)
                acc = acc + _dot(y[64 * j:64 * j + 64], w2_ref[pl.ds(r0, 128), :])
            issue(s)
            return acc
        return jax.lax.fori_loop(0, 32, body, jnp.zeros((64, 128), f32))

    def absorb(q, w2_ref, issue):
        def body(s, acc):
            ts = []
            for j in range(4):
                r0 = pl.multiple_of((32 * j + s) * 128, 128)
                ts.append(_nt_dot(q, w2_ref[pl.ds(r0, 128), :]))
            t = jnp.where(diag256, jnp.concatenate(ts, axis=0), 0.0).astype(bf16)
            g_s = (lane128 == 4 * s + (row128 >> 5)).astype(bf16)
            acc = acc + _dot(t, g_s)
            issue(s)
            return acc
        return jax.lax.fori_loop(0, 32, body, jnp.zeros((256, 128), f32))

    pltpu.make_async_copy(x_hbm, x_v, wsem.at[0]).start()
    pltpu.make_async_copy(gw_hbm, gw_v, wsem.at[1]).start()
    halves(bwq_hbm, bwq_v, wsem.at[2], 8192, 0, _pieces(8192, _P256))
    halves(wuk_hbm, wuk_v, wsem.at[3], 8192, 0, _pieces(8192, _P256))

    wait_all(x_v, wsem.at[0])
    row8 = jax.lax.broadcasted_iota(jnp.int32, (8, _DM), 0)
    x0 = x_v[0:1, :].astype(f32)
    x1 = x_v[1:2, :].astype(f32)
    x8 = jnp.where(row8 == 0, jnp.broadcast_to(x0, (8, _DM)),
                   jnp.where(row8 == 1, jnp.broadcast_to(x1, (8, _DM)), 0.0))
    row64 = jax.lax.broadcasted_iota(jnp.int32, (64, 128), 0)
    for j in range(4):
        xa = jnp.broadcast_to(x0[:, 128 * j:128 * j + 128], (64, 128))
        xb = jnp.broadcast_to(x1[:, 128 * j:128 * j + 128], (64, 128))
        stack_v[64 * j:64 * j + 64, :] = jnp.where(row64 < 32, xa, xb).astype(bf16)

    def issue_ckv(b):
        def f(s):
            lo = pl.multiple_of(s * 128, 128)
            halves(ckv_hbm, ckv_v.at[b], wsem.at[4 + b], _SK // 2, lo, _even_pieces(128, _P1K, 8),
                   src_base=b * _SK)
        return f

    wait_all(bwq_v, wsem.at[2])
    q_b = expand(stack_v[...], bwq_v, issue_ckv(0)).astype(bf16)
    wait_all(wuk_v, wsem.at[3])
    stack_v[...] = absorb(q_b, wuk_v, issue_ckv(1)).astype(bf16)

    qa = [jnp.concatenate([stack_v[64 * j + 32 * b:64 * j + 32 * b + 32, :] for j in range(4)], axis=1)
          for b in range(_B)]
    n_t = _SK // _CKV_CHUNK
    for b in range(_B):
        wait_all(ckv_v.at[b], wsem.at[4 + b])

        def bstep(t, carry, b=b):
            m, l, acc = carry
            c = ckv_v[b, pl.ds(pl.multiple_of(t * _CKV_CHUNK, _CKV_CHUNK), _CKV_CHUNK), :]
            s = _nt_dot(qa[b], c) * _SCALE
            m_new = jnp.maximum(m, jnp.max(s, axis=1, keepdims=True))
            alpha = jnp.exp(m - m_new)
            p = jnp.exp(s - m_new)
            l = alpha * l + jnp.sum(p, axis=1, keepdims=True)
            acc = alpha * acc + _dot(p.astype(bf16), c)
            if b == 0:
                halves(wuv_hbm, wuv_v, wsem.at[6], 8192, pl.multiple_of(t * (8192 // n_t), 16),
                       _even_pieces(8192 // n_t, _P256, 16))
                halves(awq_hbm, awq_v, wsem.at[8], 256, pl.multiple_of(t * (256 // n_t), 16),
                       _pieces(256 // n_t, 16))
            else:
                halves(bwo_hbm, bwo_v, wsem.at[7], 2048, pl.multiple_of(t * (2048 // n_t), 16),
                       _even_pieces(2048 // n_t, _P1K, 8))
                halves(awo_hbm, awo_v, wsem.at[9], 2048, pl.multiple_of(t * (2048 // n_t), 16),
                       _even_pieces(2048 // n_t, _P1K, 8))
            return m_new, l, acc
        init = (jnp.full((32, 1), -1e30, f32), jnp.zeros((32, 1), f32), jnp.zeros((32, _DC), f32))
        _, l, acc = jax.lax.fori_loop(0, n_t, bstep, init)
        ctx_c = (acc / l).astype(bf16)
        for j in range(4):
            stack_v[64 * j + 32 * b:64 * j + 32 * b + 32, :] = ctx_c[:, 128 * j:128 * j + 128]

    def issue_first_heads(s):
        head = s // 16
        lo = pl.multiple_of((s % 16) * 512, 512)
        for off, n in _even_pieces(512, _P256, 16):
            pltpu.make_async_copy(kc_hbm.at[pl.ds(head * _SK + lo + off, n)],
                                  kbuf.at[head, pl.ds(lo + off, n)], ksem.at[head]).start(priority=0)
            pltpu.make_async_copy(vc_hbm.at[pl.ds(head * _SK + lo + off, n)],
                                  vbuf.at[head, pl.ds(lo + off, n)], vsem.at[head]).start(priority=1)

    wait_all(wuv_v, wsem.at[6])
    ctx = expand(stack_v[...], wuv_v, issue_first_heads)

    wait_all(bwo_v, wsem.at[7])
    row8s = jax.lax.broadcasted_iota(jnp.int32, (8, 128), 0)
    out_b = jnp.zeros((8, _DM), f32)
    for h in range(_H):
        lhs = jnp.where(row8s == 0, jnp.broadcast_to(ctx[h:h + 1], (8, 128)),
                        jnp.where(row8s == 1, jnp.broadcast_to(ctx[32 + h:33 + h], (8, 128)), 0.0))
        out_b = out_b + _dot(lhs.astype(bf16), bwo_v[128 * h:128 * h + 128, :])

    wait_all(gw_v, wsem.at[1])
    gw = gw_v[...].astype(f32).reshape(1, _DM)
    g = jax.nn.sigmoid(jnp.sum(x8 * gw, axis=1, keepdims=True))
    gated_b = (1.0 - g) * out_b

    n_kv = len(kv_pieces)
    for hd in range(2, _AHEAD):
        issue_kv(hd, hd, range(n_kv // 2))
    wait_all(awq_v, wsem.at[8])
    q_a = _dot(x8.astype(bf16), awq_v[...]).astype(bf16).astype(f32)
    for b in range(_B):
        for h in range(_H):
            q3_v[b * _H + h] = jnp.broadcast_to(q_a[b:b + 1, 128 * h:128 * h + 128], (8, 128))
    acco_v[...] = jnp.zeros(acco_v.shape, f32)
    for hd in range(2, _AHEAD):
        issue_kv(hd, hd, range(n_kv // 2, n_kv))
    wait_all(awo_v, wsem.at[9])

    def head_step(i, carry, do_issue):
        slot = i % _NBUF
        b = i // _H
        h = i % _H
        q = q3_v[i].astype(bf16)
        wait_all(kbuf.at[slot], ksem.at[slot])
        s = _nt_dot(q, kbuf[slot])
        m = jnp.max(s, axis=1, keepdims=True)
        p = jnp.exp2((s - m) * (_SCALE * _LOG2E))
        l = jnp.sum(p, axis=1, keepdims=True)
        wait_all(vbuf.at[slot], vsem.at[slot])
        o = _dot(p.astype(bf16), vbuf[slot]) / l
        if do_issue:
            issue_kv(i + _AHEAD, (i + _AHEAD) % _NBUF, range(n_kv))
        wo = awo_v[pl.ds(pl.multiple_of(h * 128, 128), 128), :]
        acco_v[b] = acco_v[b] + _dot(o.astype(bf16), wo)
        return carry
    jax.lax.fori_loop(0, _NBH - _AHEAD, lambda i, c: head_step(i, c, True), 0)
    jax.lax.fori_loop(_NBH - _AHEAD, _NBH, lambda i, c: head_step(i, c, False), 0)

    out_a = jnp.where(row8 == 0, acco_v[0], acco_v[1])
    out_v[...] = (g * out_a + gated_b)[0:_B, :].astype(bf16)
    out_copy = pltpu.make_async_copy(out_v, o_hbm, osem)
    out_copy.start()
    out_copy.wait()


@jax.jit
def pallas_gated_mix__mha_block_cached__compressed_kv_cla__decode_kernel(
    A_x: jax.Array,
    A_k_cache: jax.Array,
    A_v_cache: jax.Array,
    A_wq: jax.Array,
    A_wo: jax.Array,
    B_x: jax.Array,
    B_c_kv: jax.Array,
    B_w_q: jax.Array,
    B_w_uk: jax.Array,
    B_w_uv: jax.Array,
    B_w_o: jax.Array,
    gate_w: jax.Array,
):
    del B_x
    bf16, f32 = jnp.bfloat16, jnp.float32
    x = A_x.reshape(_B, _DM)
    kc = A_k_cache.reshape(_NBH * _SK, _DH)
    vc = A_v_cache.reshape(_NBH * _SK, _DH)
    ckv = B_c_kv.reshape(_B * _SK, _DC)
    bwq = B_w_q.reshape(_DM * _H, _DH)
    wuk = B_w_uk.reshape(_DC * _H, _DH)
    wuv = B_w_uv.reshape(_DC * _H, _DH)
    bwo = B_w_o.reshape(_H * _DH, _DM)

    scratch = [
        pltpu.VMEM((_B, _DM), bf16),
        pltpu.VMEM((_DM,), bf16),
        pltpu.VMEM((_DM, _H * _DH), bf16),
        pltpu.VMEM((_H * _DH, _DM), bf16),
        pltpu.VMEM((_B, _SK, _DC), bf16),
        pltpu.VMEM((_DM * _H, _DH), bf16),
        pltpu.VMEM((_DC * _H, _DH), bf16),
        pltpu.VMEM((_DC * _H, _DH), bf16),
        pltpu.VMEM((_H * _DH, _DM), bf16),
        pltpu.VMEM((_NBUF, _SK, _DH), bf16),
        pltpu.VMEM((_NBUF, _SK, _DH), bf16),
        pltpu.VMEM((256, 128), bf16),
        pltpu.VMEM((_NBH, 8, _DH), f32),
        pltpu.VMEM((_B, 8, _DM), f32),
        pltpu.VMEM((_B, _DM), bf16),
        pltpu.SemaphoreType.DMA((10,)),
        pltpu.SemaphoreType.DMA((_NBUF,)),
        pltpu.SemaphoreType.DMA((_NBUF,)),
        pltpu.SemaphoreType.DMA(()),
    ]
    out = pl.pallas_call(
        _kernel,
        out_shape=jax.ShapeDtypeStruct((_B, _DM), bf16),
        in_specs=[pl.BlockSpec(memory_space=pl.ANY)] * 11,
        out_specs=pl.BlockSpec(memory_space=pl.ANY),
        scratch_shapes=scratch,
        compiler_params=pltpu.CompilerParams(vmem_limit_bytes=100 * 1024 * 1024),
    )(x, kc, vc, A_wq, A_wo, ckv, bwq, wuk, wuv, bwo, gate_w)
    return out.reshape(_B, 1, _DM)
```

```python
import jax
import jax.numpy as jnp
import jax.experimental.pallas as pl
import jax.experimental.pallas.tpu as pltpu

_B, _H, _SK, _DH, _DM, _DC = 2, 32, 8192, 128, 512, 512
_NBH = _B * _H
_SCALE = _DH ** -0.5
_LOG2E = 1.4426950408889634

_NBUF = 4
_AHEAD = 3
_P256 = 144
_P1K = 48
_STRIDE = 43
_CKV_CHUNK = 1024


def _pieces(total, piece):
    out, off = [], 0
    while off < total:
        n = min(piece, total - off)
        out.append((off, n))
        off += n
    return out


def _sizes(total, piece, align):
    n = -(-total // piece)
    units = total // align
    bounds = [(units * k) // n * align for k in range(n + 1)]
    return [bounds[k + 1] - bounds[k] for k in range(n)]


def _strided(pieces, stride):
    n = len(pieces)
    return [pieces[(j * stride) % n] for j in range(n)]


def _regions(step, n_steps, sizes, align):
    out, base = [], 0
    for n in sizes:
        out.append((pl.multiple_of(base + step * n, align), n))
        base += n_steps * n
    return out


def _nt_dot(a, b):
    return jax.lax.dot_general(a, b, (((1,), (1,)), ((), ())),
                               preferred_element_type=jnp.float32)


def _dot(a, b):
    return jnp.dot(a, b, preferred_element_type=jnp.float32)


def _kernel(x_hbm, kc_hbm, vc_hbm, awq_hbm, awo_hbm, ckv_hbm, bwq_hbm, wuk_hbm,
            wuv_hbm, bwo_hbm, gw_hbm, o_hbm,
            x_v, gw_v, awq_v, awo_v, ckv_v, bwq_v, wuk_v, wuv_v, bwo_v,
            kbuf, vbuf, stack_v, q3_v, acco_v, out_v, wsem, ksem, vsem, osem):
    bf16, f32 = jnp.bfloat16, jnp.float32

    def halves(src, dst, sem, half, pieces, src_base=0):
        for off, m in pieces:
            for p in range(2):
                r = off + p * half
                pltpu.make_async_copy(src.at[pl.ds(src_base + r, m)], dst.at[pl.ds(r, m)],
                                      sem).start(priority=p)

    kv_pieces = _strided(_pieces(_SK, _P256), _STRIDE)

    def issue_kv(head, slot, idxs):
        base = head * _SK
        for j in idxs:
            off, n = kv_pieces[j]
            pltpu.make_async_copy(kc_hbm.at[pl.ds(base + off, n)],
                                  kbuf.at[slot, pl.ds(off, n)], ksem.at[slot]).start(priority=0)
            pltpu.make_async_copy(vc_hbm.at[pl.ds(base + off, n)],
                                  vbuf.at[slot, pl.ds(off, n)], vsem.at[slot]).start(priority=1)

    def wait_all(dst, sem):
        pltpu.make_async_copy(dst, dst, sem).wait()

    row256 = jax.lax.broadcasted_iota(jnp.int32, (256, 128), 0)
    lane256 = jax.lax.broadcasted_iota(jnp.int32, (256, 128), 1)
    diag256 = (row256 & 31) == (lane256 & 31)
    row128 = jax.lax.broadcasted_iota(jnp.int32, (128, 128), 0)
    lane128 = jax.lax.broadcasted_iota(jnp.int32, (128, 128), 1)

    def expand(cst, w2_ref, issue):
        def body(s, acc):
            e_s = (row128 == 4 * s + (lane128 >> 5)).astype(bf16)
            y = jnp.where(diag256, _dot(cst, e_s), 0.0).astype(bf16)
            for j in range(4):
                r0 = pl.multiple_of((32 * j + s) * 128, 128)
                acc = acc + _dot(y[64 * j:64 * j + 64], w2_ref[pl.ds(r0, 128), :])
            issue(s)
            return acc
        return jax.lax.fori_loop(0, 32, body, jnp.zeros((64, 128), f32))

    def absorb(q, w2_ref, issue):
        def body(s, acc):
            ts = []
            for j in range(4):
                r0 = pl.multiple_of((32 * j + s) * 128, 128)
                ts.append(_nt_dot(q, w2_ref[pl.ds(r0, 128), :]))
            t = jnp.where(diag256, jnp.concatenate(ts, axis=0), 0.0).astype(bf16)
            g_s = (lane128 == 4 * s + (row128 >> 5)).astype(bf16)
            acc = acc + _dot(t, g_s)
            issue(s)
            return acc
        return jax.lax.fori_loop(0, 32, body, jnp.zeros((256, 128), f32))

    pltpu.make_async_copy(x_hbm, x_v, wsem.at[0]).start()
    pltpu.make_async_copy(gw_hbm, gw_v, wsem.at[1]).start()
    halves(bwq_hbm, bwq_v, wsem.at[2], 8192, _strided(_pieces(8192, _P256), _STRIDE))
    halves(wuk_hbm, wuk_v, wsem.at[3], 8192, _strided(_pieces(8192, _P256), _STRIDE))

    wait_all(x_v, wsem.at[0])
    row8 = jax.lax.broadcasted_iota(jnp.int32, (8, _DM), 0)
    x0 = x_v[0:1, :].astype(f32)
    x1 = x_v[1:2, :].astype(f32)
    x8 = jnp.where(row8 == 0, jnp.broadcast_to(x0, (8, _DM)),
                   jnp.where(row8 == 1, jnp.broadcast_to(x1, (8, _DM)), 0.0))
    row64 = jax.lax.broadcasted_iota(jnp.int32, (64, 128), 0)
    for j in range(4):
        xa = jnp.broadcast_to(x0[:, 128 * j:128 * j + 128], (64, 128))
        xb = jnp.broadcast_to(x1[:, 128 * j:128 * j + 128], (64, 128))
        stack_v[64 * j:64 * j + 64, :] = jnp.where(row64 < 32, xa, xb).astype(bf16)

    def issue_ckv(b):
        def f(s):
            halves(ckv_hbm, ckv_v.at[b], wsem.at[4 + b], _SK // 2,
                   _regions(s, 32, _sizes(128, _P1K, 8), 8), src_base=b * _SK)
        return f

    wait_all(bwq_v, wsem.at[2])
    q_b = expand(stack_v[...], bwq_v, issue_ckv(0)).astype(bf16)
    wait_all(wuk_v, wsem.at[3])
    stack_v[...] = absorb(q_b, wuk_v, issue_ckv(1)).astype(bf16)

    qa = [jnp.concatenate([stack_v[64 * j + 32 * b:64 * j + 32 * b + 32, :] for j in range(4)], axis=1)
          for b in range(_B)]
    n_t = _SK // _CKV_CHUNK
    for b in range(_B):
        wait_all(ckv_v.at[b], wsem.at[4 + b])

        def bstep(t, carry, b=b):
            m, l, acc = carry
            c = ckv_v[b, pl.ds(pl.multiple_of(t * _CKV_CHUNK, _CKV_CHUNK), _CKV_CHUNK), :]
            s = _nt_dot(qa[b], c) * _SCALE
            m_new = jnp.maximum(m, jnp.max(s, axis=1, keepdims=True))
            alpha = jnp.exp(m - m_new)
            p = jnp.exp(s - m_new)
            l = alpha * l + jnp.sum(p, axis=1, keepdims=True)
            acc = alpha * acc + _dot(p.astype(bf16), c)
            if b == 0:
                halves(wuv_hbm, wuv_v, wsem.at[6], 8192,
                       _regions(t, n_t, _sizes(8192 // n_t, _P256, 16), 16))
                halves(awq_hbm, awq_v, wsem.at[8], 256,
                       _regions(t, n_t, _sizes(256 // n_t, 16, 16), 16))
            else:
                halves(bwo_hbm, bwo_v, wsem.at[7], 2048,
                       _regions(t, n_t, _sizes(2048 // n_t, _P1K, 8), 8))
                halves(awo_hbm, awo_v, wsem.at[9], 2048,
                       _regions(t, n_t, _sizes(2048 // n_t, _P1K, 8), 8))
            return m_new, l, acc
        init = (jnp.full((32, 1), -1e30, f32), jnp.zeros((32, 1), f32), jnp.zeros((32, _DC), f32))
        _, l, acc = jax.lax.fori_loop(0, n_t, bstep, init)
        ctx_c = (acc / l).astype(bf16)
        for j in range(4):
            stack_v[64 * j + 32 * b:64 * j + 32 * b + 32, :] = ctx_c[:, 128 * j:128 * j + 128]

    def issue_first_heads(s):
        head = s // 16
        for off, n in _regions(s % 16, 16, _sizes(512, _P256, 16), 16):
            pltpu.make_async_copy(kc_hbm.at[pl.ds(head * _SK + off, n)],
                                  kbuf.at[head, pl.ds(off, n)], ksem.at[head]).start(priority=0)
            pltpu.make_async_copy(vc_hbm.at[pl.ds(head * _SK + off, n)],
                                  vbuf.at[head, pl.ds(off, n)], vsem.at[head]).start(priority=1)

    wait_all(wuv_v, wsem.at[6])
    ctx = expand(stack_v[...], wuv_v, issue_first_heads)

    wait_all(bwo_v, wsem.at[7])
    row8s = jax.lax.broadcasted_iota(jnp.int32, (8, 128), 0)
    out_b = jnp.zeros((8, _DM), f32)
    for h in range(_H):
        lhs = jnp.where(row8s == 0, jnp.broadcast_to(ctx[h:h + 1], (8, 128)),
                        jnp.where(row8s == 1, jnp.broadcast_to(ctx[32 + h:33 + h], (8, 128)), 0.0))
        out_b = out_b + _dot(lhs.astype(bf16), bwo_v[128 * h:128 * h + 128, :])

    wait_all(gw_v, wsem.at[1])
    gw = gw_v[...].astype(f32).reshape(1, _DM)
    g = jax.nn.sigmoid(jnp.sum(x8 * gw, axis=1, keepdims=True))
    gated_b = (1.0 - g) * out_b

    n_kv = len(kv_pieces)
    for hd in range(2, _AHEAD):
        issue_kv(hd, hd, range(n_kv // 2))
    wait_all(awq_v, wsem.at[8])
    q_a = _dot(x8.astype(bf16), awq_v[...]).astype(bf16).astype(f32)
    for b in range(_B):
        for h in range(_H):
            q3_v[b * _H + h] = jnp.broadcast_to(q_a[b:b + 1, 128 * h:128 * h + 128], (8, 128))
    acco_v[...] = jnp.zeros(acco_v.shape, f32)
    for hd in range(2, _AHEAD):
        issue_kv(hd, hd, range(n_kv // 2, n_kv))
    wait_all(awo_v, wsem.at[9])

    def head_step(i, carry, do_issue):
        slot = i % _NBUF
        b = i // _H
        h = i % _H
        q = q3_v[i].astype(bf16)
        wait_all(kbuf.at[slot], ksem.at[slot])
        s = _nt_dot(q, kbuf[slot])
        m = jnp.max(s, axis=1, keepdims=True)
        p = jnp.exp2((s - m) * (_SCALE * _LOG2E))
        l = jnp.sum(p, axis=1, keepdims=True)
        wait_all(vbuf.at[slot], vsem.at[slot])
        o = _dot(p.astype(bf16), vbuf[slot]) / l
        if do_issue:
            issue_kv(i + _AHEAD, (i + _AHEAD) % _NBUF, range(n_kv))
        wo = awo_v[pl.ds(pl.multiple_of(h * 128, 128), 128), :]
        acco_v[b] = acco_v[b] + _dot(o.astype(bf16), wo)
        return carry
    jax.lax.fori_loop(0, _NBH - _AHEAD, lambda i, c: head_step(i, c, True), 0)
    jax.lax.fori_loop(_NBH - _AHEAD, _NBH, lambda i, c: head_step(i, c, False), 0)

    out_a = jnp.where(row8 == 0, acco_v[0], acco_v[1])
    out_v[...] = (g * out_a + gated_b)[0:_B, :].astype(bf16)
    out_copy = pltpu.make_async_copy(out_v, o_hbm, osem)
    out_copy.start()
    out_copy.wait()


@jax.jit
def pallas_gated_mix__mha_block_cached__compressed_kv_cla__decode_kernel(
    A_x: jax.Array,
    A_k_cache: jax.Array,
    A_v_cache: jax.Array,
    A_wq: jax.Array,
    A_wo: jax.Array,
    B_x: jax.Array,
    B_c_kv: jax.Array,
    B_w_q: jax.Array,
    B_w_uk: jax.Array,
    B_w_uv: jax.Array,
    B_w_o: jax.Array,
    gate_w: jax.Array,
):
    del B_x
    bf16, f32 = jnp.bfloat16, jnp.float32
    x = A_x.reshape(_B, _DM)
    kc = A_k_cache.reshape(_NBH * _SK, _DH)
    vc = A_v_cache.reshape(_NBH * _SK, _DH)
    ckv = B_c_kv.reshape(_B * _SK, _DC)
    bwq = B_w_q.reshape(_DM * _H, _DH)
    wuk = B_w_uk.reshape(_DC * _H, _DH)
    wuv = B_w_uv.reshape(_DC * _H, _DH)
    bwo = B_w_o.reshape(_H * _DH, _DM)

    scratch = [
        pltpu.VMEM((_B, _DM), bf16),
        pltpu.VMEM((_DM,), bf16),
        pltpu.VMEM((_DM, _H * _DH), bf16),
        pltpu.VMEM((_H * _DH, _DM), bf16),
        pltpu.VMEM((_B, _SK, _DC), bf16),
        pltpu.VMEM((_DM * _H, _DH), bf16),
        pltpu.VMEM((_DC * _H, _DH), bf16),
        pltpu.VMEM((_DC * _H, _DH), bf16),
        pltpu.VMEM((_H * _DH, _DM), bf16),
        pltpu.VMEM((_NBUF, _SK, _DH), bf16),
        pltpu.VMEM((_NBUF, _SK, _DH), bf16),
        pltpu.VMEM((256, 128), bf16),
        pltpu.VMEM((_NBH, 8, _DH), f32),
        pltpu.VMEM((_B, 8, _DM), f32),
        pltpu.VMEM((_B, _DM), bf16),
        pltpu.SemaphoreType.DMA((10,)),
        pltpu.SemaphoreType.DMA((_NBUF,)),
        pltpu.SemaphoreType.DMA((_NBUF,)),
        pltpu.SemaphoreType.DMA(()),
    ]
    out = pl.pallas_call(
        _kernel,
        out_shape=jax.ShapeDtypeStruct((_B, _DM), bf16),
        in_specs=[pl.BlockSpec(memory_space=pl.ANY)] * 11,
        out_specs=pl.BlockSpec(memory_space=pl.ANY),
        scratch_shapes=scratch,
        compiler_params=pltpu.CompilerParams(vmem_limit_bytes=100 * 1024 * 1024),
    )(x, kc, vc, A_wq, A_wo, ckv, bwq, wuk, wuv, bwo, gate_w)
    return out.reshape(_B, 1, _DM)
```
